```python
import jax
import jax.numpy as jnp

def _softmax(x, axis=-1):
    return jax.nn.softmax(x, axis=axis)
def _gelu(x):
    return jax.nn.gelu(x, approximate=True)
def _silu(x):
    return jax.nn.silu(x)
def _sigmoid(x):
    return jax.nn.sigmoid(x)
def _layernorm(x, axis=-1, eps=1e-5):
    m = jnp.mean(x, axis=axis, keepdims=True)
    v = jnp.var(x, axis=axis, keepdims=True)
    return (x - m) / jnp.sqrt(v + eps)
def _scatter_add(tgt, idx, src, axis=0):
    return tgt.at[idx].add(src)
def _segment_sum(src, seg, n):
    return jax.ops.segment_sum(src, seg, n)
class _Rng:
    def __init__(self, key):
        self._k = key
    def _next(self):
        self._k, sub = jax.random.split(self._k)
        return sub
    def normal(self, shape):
        return jax.random.normal(self._next(), shape, dtype=jnp.bfloat16)
    def randint(self, lo, hi, shape):
        return jax.random.randint(self._next(), shape, lo, hi, dtype=jnp.int32)
    def uniform(self, shape, lo=0.0, hi=1.0):
        return jax.random.uniform(self._next(), shape, jnp.bfloat16, lo, hi)
    def permutation(self, n):
        return jax.random.permutation(self._next(), n)


kernel_name = 'recurrent_scan__sliding_block_cached__mixer_s_mlp__decode'

def setup_inputs():
    _rng = _Rng(jax.random.key(int.from_bytes(__import__("os").urandom(4), "little")))
    _w = (lambda a: (lambda t: t.astype(jnp.bfloat16) if jnp.issubdtype(t.dtype, jnp.floating) else t)(jnp.asarray(a)))
    def _A_setup():
        B, Sq, D = 1, 1, 512
        Hq, Hkv, Sk, Dh = 32, 32, 32768, 128
        assert Hq % Hkv == 0, (Hq, Hkv)
        return {
            "x": _w((lambda *s: _rng.normal(s) * 0.05)(B, Sq, D)),
            "k_cache": _w((lambda *s: _rng.normal(s) * 0.05)(B, Hkv, Sk, Dh)),
            "v_cache": _w((lambda *s: _rng.normal(s) * 0.05)(B, Hkv, Sk, Dh)),
            "wq": _w((lambda *s: _rng.normal(s) * 0.05)(D, Hq * Dh) * (D ** -0.5)),
            "wo": _w((lambda *s: _rng.normal(s) * 0.05)(Hq * Dh, D) * ((Hq * Dh) ** -0.5)),
        }
    _A_in = _A_setup()

    def _B_setup():
        B, S, D, F = 1, 1, 512, 1376
        return {
            "x":  _w((lambda *s: _rng.normal(s) * 0.05)(B, S, D)),
            "w1": _w((lambda *s: _rng.normal(s) * 0.05)(D, D) * (D ** -0.5)),
            "w2": _w((lambda *s: _rng.normal(s) * 0.05)(D, D) * (D ** -0.5)),
            "w3": _w((lambda *s: _rng.normal(s) * 0.05)(D, F) * (D ** -0.5)),
            "w4": _w((lambda *s: _rng.normal(s) * 0.05)(F, D) * (F ** -0.5)),
        }
    _B_in = _B_setup()

    return {
        "A_x": _A_in["x"],
        "A_k_cache": _A_in["k_cache"],
        "A_v_cache": _A_in["v_cache"],
        "A_wq": _A_in["wq"],
        "A_wo": _A_in["wo"],
        "B_x": _B_in["x"],
        "B_w1": _B_in["w1"],
        "B_w2": _B_in["w2"],
        "B_w3": _B_in["w3"],
        "B_w4": _B_in["w4"],
    }

def reference(A_x, A_k_cache, A_v_cache, A_wq, A_wo, B_x, B_w1, B_w2, B_w3, B_w4):
    def _A_ref(x, k_cache, v_cache, wq, wo):
        B, Sq, D = x.shape
        Hq, Dh = 32, 128
        Hkv, Sk = k_cache.shape[1], k_cache.shape[2]
        W = min(4096, max(256, Sk // 4))
        rep = Hq // Hkv
        q = (lambda x, *d: x.transpose(*d))((x @ wq).reshape(B, Sq, Hq, Dh), 0, 2, 1, 3)
        k = jnp.repeat(k_cache[:, :, Sk - W:, :], rep, axis=1)
        v = jnp.repeat(v_cache[:, :, Sk - W:, :], rep, axis=1)
        scores = jnp.einsum("bhqd,bhkd->bhqk", q, k) * (Dh ** -0.5)
        p = _softmax(scores, axis=-1)
        o = jnp.einsum("bhqk,bhkd->bhqd", p, v)
        return (lambda x, *d: x.transpose(*d))(o, 0, 2, 1, 3).reshape(B, Sq, Hq * Dh) @ wo

    def _B_ref(x, w1, w2, w3, w4):
        B, S, D = x.shape
        h = _gelu(_layernorm(x, axis=-1) @ w1)
        c = D // 4
        g0 = jnp.pad(h[:, :, 0*c:1*c], ((0, 0), (1, 0), (0, 0)))[:, :S, :]
        g1 = jnp.pad(h[:, :, 1*c:2*c], ((0, 0), (0, 1), (0, 0)))[:, 1:, :]
        g2 = jnp.pad(h[:, :, 2*c:3*c], ((0, 0), (2, 0), (0, 0)))[:, :S, :]
        g3 = jnp.pad(h[:, :, 3*c:   ], ((0, 0), (0, 2), (0, 0)))[:, 2:, :]
        hs = jnp.concatenate([g0, g1, g2, g3], axis=-1) @ w2
        x1 = x + hs
        h2 = _gelu(_layernorm(x1, axis=-1) @ w3) @ w4
        return x1 + h2

    x = A_x
    xn = _layernorm(x, axis=-1)
    s = _A_ref(xn, A_k_cache, A_v_cache, A_wq, A_wo)
    g = _silu(_B_ref(xn, B_w1, B_w2, B_w3, B_w4))
    return x + s * g
```

```python
import jax
import jax.numpy as jnp
import jax.experimental.pallas as pl
import jax.experimental.pallas.tpu as pltpu

_EPS = 1e-5
_ROWS = 8
_LOOK = 2


def _layernorm(x):
    m = jnp.mean(x, axis=-1, keepdims=True)
    d = x - m
    v = jnp.mean(d * d, axis=-1, keepdims=True)
    return d * jax.lax.rsqrt(v + _EPS)


def _dot(a, b):
    return jnp.dot(a, b, preferred_element_type=jnp.float32)


def _dot_nt(a, b):
    return jax.lax.dot_general(
        a, b, (((1,), (1,)), ((), ())), preferred_element_type=jnp.float32)


@jax.jit
def pallas_recurrent_scan__sliding_block_cached__mixer_s_mlp__decode_kernel(
    A_x: jax.Array,
    A_k_cache: jax.Array,
    A_v_cache: jax.Array,
    A_wq: jax.Array,
    A_wo: jax.Array,
    B_x: jax.Array,
    B_w1: jax.Array,
    B_w2: jax.Array,
    B_w3: jax.Array,
    B_w4: jax.Array,
):
    del B_x, B_w1, B_w2
    B, S, D = A_x.shape
    _, H, SK, DH = A_k_cache.shape
    assert B == 1 and S == 1 and A_wq.shape[1] == H * DH
    W = min(4096, max(256, SK // 4))
    bf16, f32 = jnp.bfloat16, jnp.float32

    def kernel(x_h, k_h, v_h, wq_h, wo_h, w3t_h, w4_h, o_ref,
               x_v, wq_v, wo_v, w3t_v, w4_v, k_v, v_v, q_v, wsem, ksem, vsem):
        cx = pltpu.make_async_copy(x_h, x_v, wsem.at[0])
        cq = pltpu.make_async_copy(wq_h, wq_v, wsem.at[1])
        co = pltpu.make_async_copy(wo_h, wo_v, wsem.at[2])
        c3 = pltpu.make_async_copy(w3t_h, w3t_v, wsem.at[3])
        c4 = pltpu.make_async_copy(w4_h, w4_v, wsem.at[4])

        def ck(h):
            return pltpu.make_async_copy(
                k_h.at[0, h, pl.ds(SK - W, W), :], k_v.at[h], ksem.at[h])

        def cv(h):
            return pltpu.make_async_copy(
                v_h.at[0, h, pl.ds(SK - W, W), :], v_v.at[h], vsem.at[h])

        cx.start()
        cq.start()
        c3.start(priority=1)
        c4.start(priority=1)
        co.start(priority=1)
        for h in range(_LOOK):
            ck(h).start()
            cv(h).start(priority=1)

        cx.wait()
        x = x_v[0].astype(f32)
        xn = _layernorm(x).astype(bf16)
        cq.wait()
        q = _dot(jnp.broadcast_to(xn, (_ROWS, D)), wq_v[...])
        for h in range(H):
            q_v[h] = q[:, h * DH:(h + 1) * DH]

        x1 = xn.astype(f32)
        x1n = jnp.broadcast_to(_layernorm(x1).astype(bf16), (_ROWS, D))
        c3.wait()
        hid = jax.nn.gelu(_dot_nt(x1n, w3t_v[...]), approximate=True)
        c4.wait()
        gate = jax.nn.silu(x1 + _dot(hid.astype(bf16), w4_v[...]))
        co.wait()

        def head(h, acc):
            ck(h).wait()

            @pl.when(h + _LOOK < H)
            def _():
                ck(h + _LOOK).start()

            s = _dot_nt(q_v[h].astype(bf16), k_v[h]) * (DH ** -0.5)
            p = jnp.exp(s - jnp.max(s, axis=-1, keepdims=True))
            l = jnp.sum(p, axis=-1, keepdims=True)
            cv(h).wait()

            @pl.when(h + _LOOK < H)
            def _():
                cv(h + _LOOK).start(priority=1)

            o = _dot(p.astype(bf16), v_v[h]) / l
            w = wo_v[pl.ds(pl.multiple_of(h * DH, DH), DH), :]
            return acc + _dot(o.astype(bf16), w)

        attn = jax.lax.fori_loop(0, H, head, jnp.zeros((_ROWS, D), f32))
        o_ref[0] = (x + (attn * gate)[0:1]).astype(o_ref.dtype)

    w3t = B_w3.T
    hbm = pl.BlockSpec(memory_space=pl.ANY)
    return pl.pallas_call(
        kernel,
        in_specs=[hbm] * 7,
        out_specs=pl.BlockSpec(memory_space=pltpu.VMEM),
        out_shape=jax.ShapeDtypeStruct(A_x.shape, A_x.dtype),
        scratch_shapes=[
            pltpu.VMEM(A_x.shape, A_x.dtype),
            pltpu.VMEM(A_wq.shape, A_wq.dtype),
            pltpu.VMEM(A_wo.shape, A_wo.dtype),
            pltpu.VMEM(w3t.shape, w3t.dtype),
            pltpu.VMEM(B_w4.shape, B_w4.dtype),
            pltpu.VMEM((H, W, DH), A_k_cache.dtype),
            pltpu.VMEM((H, W, DH), A_v_cache.dtype),
            pltpu.VMEM((H, _ROWS, DH), f32),
            pltpu.SemaphoreType.DMA((5,)),
            pltpu.SemaphoreType.DMA((H,)),
            pltpu.SemaphoreType.DMA((H,)),
        ],
        compiler_params=pltpu.CompilerParams(vmem_limit_bytes=100 << 20),
    )(A_x, A_k_cache, A_v_cache, A_wq, A_wo, w3t, B_w4)
```

```python
import jax
import jax.numpy as jnp
import jax.experimental.pallas as pl
import jax.experimental.pallas.tpu as pltpu

_EPS = 1e-5
_ROWS = 8
_KV_ROWS = 64
_W_ROWS = 16
_WQ_TILE = (8, 1024)
_SLOTS = 4
_WO_GROUPS = (8, 8, 8, 4, 4)


def _layernorm(x):
    m = jnp.mean(x, axis=-1, keepdims=True)
    d = x - m
    v = jnp.mean(d * d, axis=-1, keepdims=True)
    return d * jax.lax.rsqrt(v + _EPS)


def _dot(a, b):
    return jnp.dot(a, b, preferred_element_type=jnp.float32)


def _dot_nt(a, b):
    return jax.lax.dot_general(
        a, b, (((1,), (1,)), ((), ())), preferred_element_type=jnp.float32)


@jax.jit
def pallas_recurrent_scan__sliding_block_cached__mixer_s_mlp__decode_kernel(
    A_x: jax.Array,
    A_k_cache: jax.Array,
    A_v_cache: jax.Array,
    A_wq: jax.Array,
    A_wo: jax.Array,
    B_x: jax.Array,
    B_w1: jax.Array,
    B_w2: jax.Array,
    B_w3: jax.Array,
    B_w4: jax.Array,
):
    del B_x, B_w1, B_w2
    B, S, D = A_x.shape
    _, H, SK, DH = A_k_cache.shape
    assert B == 1 and S == 1 and A_wq.shape[1] == H * DH
    W = min(4096, max(256, SK // 4))
    bf16, f32 = jnp.bfloat16, jnp.float32

    F = B_w4.shape[0]
    assert sum(_WO_GROUPS) == H and F % _W_ROWS == 0 and W % (2 * _KV_ROWS) == 0
    first_head = [sum(_WO_GROUPS[:g]) for g in range(len(_WO_GROUPS))]

    def kernel(x_h, k_h, v_h, wq_h, wo_h, w3t_h, w4_h, o_ref,
               x_v, wq_v, wo_v, w3t_v, w4_v, kv_v, q_v, o_v,
               wsem, ksem, vsem, osem):
        def start(src, dst, sem, queue):
            pltpu.make_async_copy(src, dst, sem).start(priority=queue)

        def wait(dst, sem):
            pltpu.make_async_copy(dst, dst, sem).wait()

        def kv(h, t):
            return kv_v.at[(h % _SLOTS) * 2 + t]

        def start_kv(h, lo=0, hi=W):
            for r in range(lo, hi, _KV_ROWS):
                src = pl.ds(SK - W + r, _KV_ROWS)
                dst = pl.ds(r, _KV_ROWS)
                start(k_h.at[0, h, src], kv(h, 0).at[dst], ksem.at[h], 0)
                start(v_h.at[0, h, src], kv(h, 1).at[dst], vsem.at[h], 1)

        def wait_kv(h):
            wait(kv(h, 0), ksem.at[h])
            wait(kv(h, 1), vsem.at[h])

        def start_wo(g):
            half = _WO_GROUPS[g] * DH // 2

            @pl.loop(0, half // _W_ROWS)
            def _(i):
                for t in range(2):
                    r = first_head[g] * DH + t * half + i * _W_ROWS
                    rows = pl.ds(pl.multiple_of(r, _W_ROWS), _W_ROWS)
                    start(wo_h.at[rows], wo_v.at[rows], osem.at[g], t)

        start(x_h, x_v, wsem.at[0], 0)

        @pl.loop(0, D // 2 // _WQ_TILE[0])
        def _(i):
            for c in range(0, H * DH, _WQ_TILE[1]):
                for t in range(2):
                    r = pl.multiple_of(t * (D // 2) + i * _WQ_TILE[0], _WQ_TILE[0])
                    idx = (pl.ds(r, _WQ_TILE[0]), pl.ds(c, _WQ_TILE[1]))
                    start(wq_h.at[idx], wq_v.at[idx], wsem.at[1], t)

        @pl.loop(0, F // _W_ROWS)
        def _(i):
            rows = pl.ds(pl.multiple_of(i * _W_ROWS, _W_ROWS), _W_ROWS)
            start(w3t_h.at[rows], w3t_v.at[rows], wsem.at[2], 0)
            start(w4_h.at[rows], w4_v.at[rows], wsem.at[3], 1)

        wait(x_v, wsem.at[0])
        x = x_v[0].astype(f32)
        xn = _layernorm(x).astype(bf16)
        wait(wq_v, wsem.at[1])
        start_kv(0)
        q = _dot(jnp.broadcast_to(xn, (_ROWS, D)), wq_v[...])
        for h in range(H):
            q_v[h] = q[:, h * DH:(h + 1) * DH]

        x1 = xn.astype(f32)
        x1n = jnp.broadcast_to(_layernorm(x1).astype(bf16), (_ROWS, D))
        wait(w3t_v, wsem.at[2])
        wait(w4_v, wsem.at[3])
        start_kv(1)
        hid = jax.nn.gelu(_dot_nt(x1n, w3t_v[...]), approximate=True)
        gate = jax.nn.silu(x1 + _dot(hid.astype(bf16), w4_v[...]))

        def attend(h, between=lambda: None):
            s = _dot_nt(q_v[h].astype(bf16), kv(h, 0)[...]) * (DH ** -0.5)
            p = jnp.exp(s - jnp.max(s, axis=-1, keepdims=True))
            l = jnp.sum(p, axis=-1, keepdims=True)
            between()
            o_v[h] = _dot(p.astype(bf16), kv(h, 1)[...]) / l

        @pl.loop(0, H - 2)
        def _(h):
            wait_kv(h)
            start_kv(h + 2, 0, W // 2)
            attend(h, lambda: start_kv(h + 2, W // 2, W))

        @pl.loop(H - 2, H)
        def _(h):
            wait_kv(h)

            @pl.when(h == H - 2)
            def _():
                for g in range(2):
                    start_wo(g)

            @pl.when(h == H - 1)
            def _():
                for g in range(2, len(_WO_GROUPS)):
                    start_wo(g)

            attend(h)

        attn = jnp.zeros((_ROWS, D), f32)
        for g, (h0, n) in enumerate(zip(first_head, _WO_GROUPS)):
            o = jnp.concatenate([o_v[h0 + i] for i in range(n)], axis=1)
            w = wo_v.at[pl.ds(h0 * DH, n * DH)]
            wait(w, osem.at[g])
            attn = attn + _dot(o.astype(bf16), w[...])
        o_ref[0] = (x + (attn * gate)[0:1]).astype(o_ref.dtype)

    w3t = B_w3.T
    hbm = pl.BlockSpec(memory_space=pl.ANY)
    return pl.pallas_call(
        kernel,
        in_specs=[hbm] * 7,
        out_specs=pl.BlockSpec(memory_space=pltpu.VMEM),
        out_shape=jax.ShapeDtypeStruct(A_x.shape, A_x.dtype),
        scratch_shapes=[
            pltpu.VMEM(A_x.shape, A_x.dtype),
            pltpu.VMEM(A_wq.shape, A_wq.dtype),
            pltpu.VMEM(A_wo.shape, A_wo.dtype),
            pltpu.VMEM(w3t.shape, w3t.dtype),
            pltpu.VMEM(B_w4.shape, B_w4.dtype),
            pltpu.VMEM((2 * _SLOTS, W, DH), A_k_cache.dtype),
            pltpu.VMEM((H, _ROWS, DH), f32),
            pltpu.VMEM((H, _ROWS, DH), f32),
            pltpu.SemaphoreType.DMA((4,)),
            pltpu.SemaphoreType.DMA((H,)),
            pltpu.SemaphoreType.DMA((H,)),
            pltpu.SemaphoreType.DMA((len(_WO_GROUPS),)),
        ],
        compiler_params=pltpu.CompilerParams(vmem_limit_bytes=100 << 20),
    )(A_x, A_k_cache, A_v_cache, A_wq, A_wo, w3t, B_w4)
```

```python
import jax
import jax.numpy as jnp
import jax.experimental.pallas as pl
import jax.experimental.pallas.tpu as pltpu

_EPS = 1e-5
_ROWS = 8
_KV_ROWS = 64
_W_ROWS = 16
_WQ_TILE = (8, 1024)
_SLOTS = 4
_WO_GROUPS = (8, 8, 12, 4)


def _layernorm(x):
    m = jnp.mean(x, axis=-1, keepdims=True)
    d = x - m
    v = jnp.mean(d * d, axis=-1, keepdims=True)
    return d * jax.lax.rsqrt(v + _EPS)


def _dot(a, b):
    return jnp.dot(a, b, preferred_element_type=jnp.float32)


def _dot_nt(a, b):
    return jax.lax.dot_general(
        a, b, (((1,), (1,)), ((), ())), preferred_element_type=jnp.float32)


@jax.jit
def pallas_recurrent_scan__sliding_block_cached__mixer_s_mlp__decode_kernel(
    A_x: jax.Array,
    A_k_cache: jax.Array,
    A_v_cache: jax.Array,
    A_wq: jax.Array,
    A_wo: jax.Array,
    B_x: jax.Array,
    B_w1: jax.Array,
    B_w2: jax.Array,
    B_w3: jax.Array,
    B_w4: jax.Array,
):
    del B_x, B_w1, B_w2
    B, S, D = A_x.shape
    _, H, SK, DH = A_k_cache.shape
    assert B == 1 and S == 1 and A_wq.shape[1] == H * DH
    W = min(4096, max(256, SK // 4))
    bf16, f32 = jnp.bfloat16, jnp.float32

    F = B_w4.shape[0]
    assert len(_WO_GROUPS) == 4 and H % 2 == 0
    assert sum(_WO_GROUPS) == H and F % _W_ROWS == 0 and W % (2 * _KV_ROWS) == 0
    first_head = [sum(_WO_GROUPS[:g]) for g in range(len(_WO_GROUPS))]

    def kernel(x_h, k_h, v_h, wq_h, wo_h, w3t_h, w4_h, o_ref,
               x_v, wq_v, wo_v, w3t_v, w4_v, kv_v, q_v, o_v, sem):
        def osem(g):
            return sem.at[(g + 2) % 4]

        def start(src, dst, sem, queue):
            pltpu.make_async_copy(src, dst, sem).start(priority=queue)

        def wait(dst, sem):
            pltpu.make_async_copy(dst, dst, sem).wait()

        def kv(h, t):
            return kv_v.at[(h % _SLOTS) * 2 + t]

        def start_kv(h, lo=0, hi=W):
            for r in range(lo, hi, _KV_ROWS):
                src = pl.ds(SK - W + r, _KV_ROWS)
                dst = pl.ds(r, _KV_ROWS)
                start(k_h.at[0, h, src], kv(h, 0).at[dst], sem.at[h % 2], 0)
                start(v_h.at[0, h, src], kv(h, 1).at[dst], sem.at[h % 2], 1)

        def wait_kv(h):
            wait(kv_v.at[pl.ds((h % _SLOTS) * 2, 2)], sem.at[h % 2])

        def start_wo(g):
            half = _WO_GROUPS[g] * DH // 2

            @pl.loop(0, half // _W_ROWS)
            def _(i):
                for t in range(2):
                    r = first_head[g] * DH + t * half + i * _W_ROWS
                    rows = pl.ds(pl.multiple_of(r, _W_ROWS), _W_ROWS)
                    start(wo_h.at[rows], wo_v.at[rows], osem(g), t)

        start(x_h, x_v, sem.at[2], 0)

        @pl.loop(0, D // 2 // _WQ_TILE[0])
        def _(i):
            for c in range(0, H * DH, _WQ_TILE[1]):
                for t in range(2):
                    r = pl.multiple_of(t * (D // 2) + i * _WQ_TILE[0], _WQ_TILE[0])
                    idx = (pl.ds(r, _WQ_TILE[0]), pl.ds(c, _WQ_TILE[1]))
                    start(wq_h.at[idx], wq_v.at[idx], sem.at[2], t)

        @pl.loop(0, F // _W_ROWS)
        def _(i):
            rows = pl.ds(pl.multiple_of(i * _W_ROWS, _W_ROWS), _W_ROWS)
            start(w3t_h.at[rows], w3t_v.at[rows], sem.at[3], 0)
            start(w4_h.at[rows], w4_v.at[rows], sem.at[3], 1)

        wait(x_v, sem.at[2])
        wait(wq_v, sem.at[2])
        start_kv(0)
        x = x_v[0].astype(f32)
        xn = _layernorm(x).astype(bf16)
        q = _dot(jnp.broadcast_to(xn, (_ROWS, D)), wq_v[...])
        for h in range(H):
            q_v[h] = q[:, h * DH:(h + 1) * DH]

        x1 = xn.astype(f32)
        x1n = jnp.broadcast_to(_layernorm(x1).astype(bf16), (_ROWS, D))
        wait(w3t_v, sem.at[3])
        wait(w4_v, sem.at[3])
        start_kv(1)
        hid = jax.nn.gelu(_dot_nt(x1n, w3t_v[...]), approximate=True)
        gate = jax.nn.silu(x1 + _dot(hid.astype(bf16), w4_v[...]))

        def attend(h, between=lambda: None):
            s = _dot_nt(q_v[h].astype(bf16), kv(h, 0)[...]) * (DH ** -0.5)
            p = jnp.exp(s - jnp.max(s, axis=-1, keepdims=True))
            l = jnp.sum(p, axis=-1, keepdims=True)
            between()
            o_v[h] = _dot(p.astype(bf16), kv(h, 1)[...]) / l

        @pl.loop(0, H - 2)
        def _(h):
            wait_kv(h)
            start_kv(h + 2, 0, W // 2)
            attend(h, lambda: start_kv(h + 2, W // 2, W))

        @pl.loop(H - 2, H)
        def _(h):
            wait_kv(h)

            @pl.when(h == H - 2)
            def _():
                for g in range(2):
                    start_wo(g)

            @pl.when(h == H - 1)
            def _():
                for g in range(2, len(_WO_GROUPS)):
                    start_wo(g)

            attend(h)

        attn = jnp.zeros((_ROWS, D), f32)
        for g, (h0, n) in enumerate(zip(first_head, _WO_GROUPS)):
            o = jnp.concatenate([o_v[h0 + i] for i in range(n)], axis=1)
            w = wo_v.at[pl.ds(h0 * DH, n * DH)]
            wait(w, osem(g))
            attn = attn + _dot(o.astype(bf16), w[...])
        o_ref[0] = (x + (attn * gate)[0:1]).astype(o_ref.dtype)

    w3t = B_w3.T
    hbm = pl.BlockSpec(memory_space=pl.ANY)
    return pl.pallas_call(
        kernel,
        in_specs=[hbm] * 7,
        out_specs=pl.BlockSpec(memory_space=pltpu.VMEM),
        out_shape=jax.ShapeDtypeStruct(A_x.shape, A_x.dtype),
        scratch_shapes=[
            pltpu.VMEM(A_x.shape, A_x.dtype),
            pltpu.VMEM(A_wq.shape, A_wq.dtype),
            pltpu.VMEM(A_wo.shape, A_wo.dtype),
            pltpu.VMEM(w3t.shape, w3t.dtype),
            pltpu.VMEM(B_w4.shape, B_w4.dtype),
            pltpu.VMEM((2 * _SLOTS, W, DH), A_k_cache.dtype),
            pltpu.VMEM((H, _ROWS, DH), f32),
            pltpu.VMEM((H, _ROWS, DH), f32),
            pltpu.SemaphoreType.DMA((4,)),
        ],
        compiler_params=pltpu.CompilerParams(vmem_limit_bytes=100 << 20),
    )(A_x, A_k_cache, A_v_cache, A_wq, A_wo, w3t, B_w4)
```
